```python
import os as _os
_os.environ.setdefault("JAX_PLATFORMS", "cpu")
import jax
import jax.numpy as jnp

def _softmax(x, axis=-1):
    return jax.nn.softmax(x, axis=axis)
def _gelu(x):
    return jax.nn.gelu(x, approximate=True)
def _silu(x):
    return jax.nn.silu(x)
def _sigmoid(x):
    return jax.nn.sigmoid(x)
def _layernorm(x, axis=-1, eps=1e-5):
    m = jnp.mean(x, axis=axis, keepdims=True)
    v = jnp.var(x, axis=axis, keepdims=True)
    return (x - m) / jnp.sqrt(v + eps)
def _scatter_add(tgt, idx, src, axis=0):
    return tgt.at[idx].add(src)
def _segment_sum(src, seg, n):
    return jax.ops.segment_sum(src, seg, n)
class _Rng:
    def __init__(self, key):
        self._k = key
    def _next(self):
        self._k, sub = jax.random.split(self._k)
        return sub
    def normal(self, shape):
        return jax.random.normal(self._next(), shape, dtype=jnp.bfloat16)
    def randint(self, lo, hi, shape):
        return jax.random.randint(self._next(), shape, lo, hi, dtype=jnp.int32)
    def uniform(self, shape, lo=0.0, hi=1.0):
        return jax.random.uniform(self._next(), shape, jnp.bfloat16, lo, hi)
    def permutation(self, n):
        return jax.random.permutation(self._next(), n)


kernel_name = 'concat_heads__sliding_block__grouped_kv_mqa__prompt'

def setup_inputs():
    _rng = _Rng(jax.random.key(int.from_bytes(__import__("os").urandom(4), "little")))
    _w = (lambda a: (lambda t: t.astype(jnp.bfloat16) if jnp.issubdtype(t.dtype, jnp.floating) else t)(jnp.asarray(a)))
    def _A_setup():
        B, S, D = 1, 2048, 576
        return {
            "x": _w((lambda *s: _rng.normal(s) * 0.2)(B, S, D)),
            "wqkv": _w((lambda *s: _rng.normal(s) * 0.2)(D, 3 * D)),
            "wo": _w((lambda *s: _rng.normal(s) * 0.05)(D, D)),
        }
    _A_in = _A_setup()

    def _B_setup():
        B, S, D, H = 1, 2048, 576, 32
        Dh = D // H
        return {
            "x": _w((lambda *s: _rng.normal(s) * 0.05)(B, S, D)),
            "wq": _w((lambda *s: _rng.normal(s) * 1.6)(D, H * Dh)),
            "wk": _w((lambda *s: _rng.normal(s) * 1.6)(D, Dh)),
            "wv": _w((lambda *s: _rng.normal(s) * 0.1)(D, Dh)),
            "wo": _w((lambda *s: _rng.normal(s) * 0.1)(H * Dh, D)),
        }
    _B_in = _B_setup()

    return {
        "A_x": _A_in["x"],
        "A_wqkv": _A_in["wqkv"],
        "A_wo": _A_in["wo"],
        "B_x": _B_in["x"],
        "B_wq": _B_in["wq"],
        "B_wk": _B_in["wk"],
        "B_wv": _B_in["wv"],
        "B_wo": _B_in["wo"],
    }

def reference(A_x, A_wqkv, A_wo, B_x, B_wq, B_wk, B_wv, B_wo):
    def _A_ref(x, wqkv, wo):
        B, S, D = x.shape
        H = 32; Dh = D // H; W = 256
        qkv = (lambda x, *d: x.transpose(*d))((x @ wqkv).reshape(B, S, 3, H, Dh), 2, 0, 3, 1, 4)
        q, k, v = qkv[0], qkv[1], qkv[2]
        scores = jnp.einsum("bhqd,bhkd->bhqk", q, k) * (Dh ** -0.5)
        idx = jnp.arange(S)
        mask = (idx[:, None] - idx[None, :] >= 0) & (idx[:, None] - idx[None, :] < W)
        scores = jnp.where(mask[None, None], scores, -1e9)
        p = _softmax(scores, axis=-1)
        o = jnp.einsum("bhqk,bhkd->bhqd", p, v)
        return (lambda x, *d: x.transpose(*d))(o, 0, 2, 1, 3).reshape(B, S, D) @ wo

    def _B_ref(x, wq, wk, wv, wo):
        B, S, D = x.shape
        H = 32
        Dh = D // H
        q = (lambda x, *d: x.transpose(*d))((x @ wq).reshape(B, S, H, Dh), 0, 2, 1, 3)
        k = x @ wk
        v = x @ wv
        scores = jnp.einsum("bhqd,bkd->bhqk", q, k) * (Dh ** -0.5)
        p = _softmax(scores, axis=-1)
        o = jnp.einsum("bhqk,bkd->bhqd", p, v)
        return (lambda x, *d: x.transpose(*d))(o, 0, 2, 1, 3).reshape(B, S, H * Dh) @ wo

    a = _A_ref(A_x, A_wqkv, A_wo)
    b = _B_ref(B_x, B_wq, B_wk, B_wv, B_wo)
    return jnp.concatenate([a, b], axis=-1)
```

```python
import functools
import numpy as np
import jax
import jax.numpy as jnp
from jax import lax
from jax.experimental import pallas as pl
from jax.experimental.pallas import tpu as pltpu

S = 2048
D = 576
H = 32
DH = 18
WIN = 256
G = 8
QB = 512
NQB = S // QB
NT = QB // 128
KC = 256
NC = S // KC
LOG2E = 1.4426950408889634
R0 = (0, 16, 32, 48)
OFF = (0, 2, 4, 6)
SHIFT = 64.0
LMIN = 2.0 ** -6
BIG = 3.0e38
f32 = jnp.float32
bf16 = jnp.bfloat16


def _rows(n, m):
    return lax.broadcasted_iota(jnp.int32, (n, m), 0)


def _lanes(n, m):
    return lax.broadcasted_iota(jnp.int32, (n, m), 1)


def _bf(x):
    return x.astype(bf16).astype(f32)


def _pv(v, p):
    return lax.dot_general(v, p, (((1,), (0,)), ((), ())), preferred_element_type=f32)


def _merge(n):
    N = n[0].shape[1]
    row = _rows(8, N)
    return jnp.concatenate([
        n[0][0:16],
        jnp.where(row < 2, n[0][16:24], n[1][0:8]),
        n[1][8:16],
        jnp.where(row < 4, n[1][16:24], n[2][0:8]),
        n[2][8:16],
        jnp.where(row < 6, n[2][16:24], n[3][0:8]),
        n[3][8:24],
    ], axis=0)


def _lrow(j):
    return (OFF[j] + DH) % 24


def _norm(acc, j):
    r1 = _lrow(j)
    return acc * (1.0 / acc[r1:r1 + 1, :])


def kernel(scale, xa_hbm, wqkv_hbm, woa_hbm, xb_hbm, wq_hbm, wkT_hbm, wvT_hbm, wob_hbm, out_hbm,
           xa_v, xb_v, wqkv_v, wq_v, woa_v, wob_v, wkT_v, wvT_v,
           wqkvT, wqT, woaT, wobT, qta, qtb, kpa, va, kb, vb, kma, kv24, ota, otb, bad, obuf,
           in_sem, out_sem):
    c = scale * LOG2E

    def cols(sb):
        return pl.ds(pl.multiple_of(sb * QB, QB), QB)

    def cp_xb(sb):
        return pltpu.make_async_copy(xb_hbm.at[:, cols(sb)], xb_v.at[:, cols(sb)], in_sem.at[sb])

    def cp_xa(sb):
        return pltpu.make_async_copy(xa_hbm.at[:, cols(sb)], xa_v.at[:, cols(sb)], in_sem.at[NQB + sb])

    whole = [pltpu.make_async_copy(s_, d_, in_sem.at[2 * NQB + i]) for i, (s_, d_) in enumerate(
        [(wq_hbm, wq_v), (wkT_hbm, wkT_v), (wvT_hbm, wvT_v), (wqkv_hbm, wqkv_v), (woa_hbm, woa_v), (wob_hbm, wob_v)])]
    cp_wq, cp_wk, cp_wv, cp_wqkv, cp_woa, cp_wob = whole
    cp_wq.start()
    cp_xb(0).start()
    cp_wk.start()
    cp_wv.start()
    cp_xb(1).start()
    cp_wqkv.start()
    cp_xb(2).start()
    cp_xb(3).start()
    cp_woa.start()
    cp_wob.start()
    for sb in range(NQB):
        cp_xa(sb).start()

    kpa[:, 0:WIN, :] = jnp.zeros((G, WIN, 128), bf16)
    va[:, :, :, 0:WIN] = jnp.zeros((G, 4, 24, WIN), f32)
    kma[...] = jnp.zeros(kma.shape, f32)
    kv24[...] = jnp.zeros(kv24.shape, f32)
    bad[...] = jnp.zeros(bad.shape, f32)
    row24 = _rows(24, QB)

    def proj_b(sb):
        cs = cols(sb)
        xb = xb_v[:, cs]
        qtb[:, cs] = jnp.dot(wqT[...], xb, preferred_element_type=f32) * c
        kv24[0, 0:DH, :] = _bf(jnp.dot(wkT_v[...], xb, preferred_element_type=f32))
        kv24[1, 0:DH, :] = _bf(jnp.dot(wvT_v[...], xb, preferred_element_type=f32))
        k24 = kv24[0]
        v24 = kv24[1]
        kaug = jnp.where(row24 == DH, 1.0, k24)
        blk = jnp.concatenate([kaug, jnp.zeros((104, QB), f32)], axis=0).astype(bf16)
        kb[cs, :] = blk.T
        n2 = jnp.max(jnp.sum(k24 * k24, axis=0, keepdims=True), axis=1, keepdims=True)
        kma[G, 0:1, :] = jnp.maximum(kma[G, 0:1, :], jnp.broadcast_to(n2, (1, 128)))
        v1 = jnp.where(row24 == DH, 1.0, v24)
        for j in range(4):
            vb[j, :, cs] = v1 if OFF[j] == 0 else pltpu.roll(v1, OFF[j], 0)

    cp_wq.wait()
    wqT[...] = wq_v[...].T
    cp_wk.wait()
    cp_wv.wait()
    cp_xb(0).wait()
    proj_b(0)
    cp_xb(1).wait()
    proj_b(1)
    cp_wqkv.wait()
    cp_xb(2).wait()
    wqkvT[...] = wqkv_v[...].T
    proj_b(2)
    cp_xb(3).wait()
    cp_woa.wait()
    cp_wob.wait()
    woaT[...] = woa_v[...].T
    wobT[...] = wob_v[...].T
    proj_b(3)

    def proj_a(sb, carry):
        cp_xa(sb).wait()
        cs = cols(sb)
        csp = pl.ds(pl.multiple_of(sb * QB + WIN, 128), QB)
        xa = xa_v[:, cs]
        qta[:, cs] = jnp.dot(wqkvT[0:D, :], xa, preferred_element_type=f32) * c
        ka = _bf(jnp.dot(wqkvT[D:2 * D, :], xa, preferred_element_type=f32))
        one8 = jnp.where(_rows(8, QB) < 1, 1.0, 0.0).astype(f32)
        for g in range(G):
            kg = ka[72 * g:72 * g + 72]
            blk = jnp.concatenate([kg, one8, jnp.zeros((48, QB), f32)], axis=0).astype(bf16)
            kpa[g, csp, :] = blk.T
            sq = kg * kg
            for j in range(4):
                w = jnp.where((row24 >= OFF[j]) & (row24 < OFF[j] + DH), sq[R0[j]:R0[j] + 24], 0.0)
                n2 = jnp.max(jnp.sum(w, axis=0, keepdims=True), axis=1, keepdims=True)
                kma[g, j:j + 1, :] = jnp.maximum(kma[g, j:j + 1, :], jnp.broadcast_to(n2, (1, 128)))
        vaT = _bf(jnp.dot(wqkvT[2 * D:3 * D, :], xa, preferred_element_type=f32))
        for g in range(G):
            for j in range(4):
                r = 72 * g + R0[j]
                va[g, j, :, csp] = jnp.where(row24 == _lrow(j), 1.0, vaT[r:r + 24])
        return carry

    lax.fori_loop(0, NQB, proj_a, 0)

    tri = _rows(128, 128) - _lanes(128, 128)

    def qa_win(qb, g, j):
        qwin = qta[pl.ds(pl.multiple_of(72 * g + R0[j], 8), 24), cols(qb)]
        return jnp.where((row24 >= OFF[j]) & (row24 < OFF[j] + DH), qwin, 0.0)

    def qb_win(qb, g, j):
        qwin = qtb[pl.ds(pl.multiple_of(72 * g + R0[j], 8), 24), cols(qb)]
        if OFF[j]:
            qwin = pltpu.roll(qwin, 24 - OFF[j], 0)
        return jnp.where(row24 < DH, qwin, 0.0)

    def wa_from(qm, j, mrow):
        parts = []
        if R0[j]:
            parts.append(jnp.zeros((R0[j], QB), f32))
        parts.append(qm)
        if 72 - R0[j] - 24:
            parts.append(jnp.zeros((72 - R0[j] - 24, QB), f32))
        parts += [mrow, jnp.zeros((48, QB), f32)]
        return jnp.concatenate(parts, axis=0).astype(bf16)

    def build_wa(qb, g, j):
        qm = qa_win(qb, g, j)
        km = jnp.concatenate([kma[g, j:j + 1, :]] * NT, axis=1)
        m = jnp.sqrt(jnp.sum(qm * qm, axis=0, keepdims=True) * km) * 1.01 - SHIFT
        return wa_from(qm, j, jnp.where(_rows(8, QB) == 0, -m, 0.0))

    def build_wb(qb, g, j):
        qm = qb_win(qb, g, j)
        km = jnp.concatenate([kma[G, 0:1, :]] * NT, axis=1)
        m = jnp.sqrt(jnp.sum(qm * qm, axis=0, keepdims=True) * km) * 1.01 - SHIFT
        qm = jnp.where(row24 == DH, -m, qm)
        return jnp.concatenate([qm, jnp.zeros((104, QB), f32)], axis=0).astype(bf16)

    def check(acc, j):
        n = acc.shape[1]
        thr = jnp.where(_rows(24, n) == _lrow(j), LMIN, -BIG)
        b = jnp.where((acc >= thr) & (acc <= BIG), 0.0, 1.0)
        r = b[0:8] + b[8:16] + b[16:24]
        return r

    def group(qb, g):
        q0 = pl.multiple_of(qb * QB, QB)
        rows = pl.ds(pl.multiple_of(72 * g, 8), 72)
        st = {}
        steps = []
        for j in range(4):
            for cc in range(NC):
                def qk(j=j, cc=cc):
                    if cc == 0:
                        st['wb', j] = build_wb(qb, g, j)
                    return jnp.dot(kb[cc * KC:(cc + 1) * KC, :], st['wb', j], preferred_element_type=f32)

                def post(s):
                    return jnp.exp2(s).astype(bf16)

                def pvf(p, j=j, cc=cc):
                    o = _pv(vb[j, :, cc * KC:(cc + 1) * KC], p)
                    st['accb', j] = o if cc == 0 else st['accb', j] + o
                    if cc == NC - 1:
                        st['nb', j] = _norm(st['accb', j], j)
                        st['chk', j] = check(st['accb', j], j)
                        if j == 3:
                            otb[rows, :] = _merge([st['nb', i] for i in range(4)])
                            bad[...] = bad[...] + (st['chk', 0] + st['chk', 1]) + (st['chk', 2] + st['chk', 3])
                steps.append((qk, post, pvf))
        for t in range(NT):
            def qk(t=t):
                if t == 0:
                    st['wa'] = [build_wa(qb, g, j) for j in range(4)]
                k0 = pl.multiple_of(q0 + 128 * t, 128)
                w = jnp.concatenate([st['wa'][j][:, 128 * t:128 * t + 128] for j in range(4)], axis=1)
                return jnp.dot(kpa[g, pl.ds(k0, 384), :], w, preferred_element_type=f32)

            def post(s):
                ps = []
                for j in range(4):
                    e = jnp.exp2(s[:, 128 * j:128 * j + 128])
                    ps.append(jnp.concatenate([jnp.where(tri > 0, e[0:128], 0.0), e[128:256],
                                               jnp.where(tri <= 0, e[256:384], 0.0)], axis=0).astype(bf16))
                return ps

            def pvf(p, t=t):
                k0 = pl.multiple_of(q0 + 128 * t, 128)
                chk = None
                for j in range(4):
                    acc = _pv(va[g, j, :, pl.ds(k0, 384)], p[j])
                    st['oa', j, t] = _norm(acc, j)
                    ck = check(acc, j)
                    chk = ck if chk is None else chk + ck
                ota[rows, 128 * t:128 * t + 128] = _merge([st['oa', j, t] for j in range(4)])
                bad[:, 128 * t:128 * t + 128] = bad[:, 128 * t:128 * t + 128] + chk
            steps.append((qk, post, pvf))
        s = steps[0][0]()
        for i in range(len(steps)):
            p = steps[i][1](s)
            if i + 1 < len(steps):
                s = steps[i + 1][0]()
            steps[i][2](p)

    def slow_group(qb, g):
        q0 = qb * QB
        rows = pl.ds(pl.multiple_of(72 * g, 8), 72)
        nb, na = [], []
        for j in range(4):
            wb = jnp.concatenate([qb_win(qb, g, j), jnp.zeros((104, QB), f32)], axis=0).astype(bf16)

            def sb_(cc, wb=wb):
                return jnp.dot(kb[pl.ds(pl.multiple_of(cc * KC, KC), KC), :], wb, preferred_element_type=f32)

            m = lax.fori_loop(0, NC, lambda cc, m: jnp.maximum(m, jnp.max(sb_(cc), axis=0, keepdims=True)),
                              jnp.full((1, QB), -jnp.inf, f32))
            acc = lax.fori_loop(
                0, NC,
                lambda cc, a, j=j, m=m: a + _pv(vb[j, :, pl.ds(pl.multiple_of(cc * KC, KC), KC)],
                                                jnp.exp2(sb_(cc) - m).astype(bf16)),
                jnp.zeros((24, QB), f32))
            nb.append(_norm(acc, j))
            wa = wa_from(qa_win(qb, g, j), j, jnp.zeros((8, QB), f32))

            def sa_(cc, wa=wa):
                s = jnp.dot(kpa[g, pl.ds(pl.multiple_of(cc * KC + WIN, KC), KC), :], wa,
                            preferred_element_type=f32)
                dist = (q0 - cc * KC) + _lanes(KC, QB) - _rows(KC, QB)
                return jnp.where((dist >= 0) & (dist < WIN), s, -1e9 * LOG2E)

            m = lax.fori_loop(0, NC, lambda cc, m: jnp.maximum(m, jnp.max(sa_(cc), axis=0, keepdims=True)),
                              jnp.full((1, QB), -jnp.inf, f32))
            acc = lax.fori_loop(
                0, NC,
                lambda cc, a, j=j, m=m: a + _pv(va[g, j, :, pl.ds(pl.multiple_of(cc * KC + WIN, KC), KC)],
                                                jnp.exp2(sa_(cc) - m).astype(bf16)),
                jnp.zeros((24, QB), f32))
            na.append(_norm(acc, j))
        otb[rows, :] = _merge(nb)
        ota[rows, :] = _merge(na)

    def cp_out(qb, slot):
        return pltpu.make_async_copy(obuf.at[slot], out_hbm.at[pl.ds(pl.multiple_of(qb * QB, QB), QB), :],
                                     out_sem.at[slot])

    def qblock(qb, carry):
        def gl(g, carry2):
            group(qb, g)
            return carry2
        lax.fori_loop(0, G, gl, 0)

        @pl.when(jnp.max(bad[...]) > 0.0)
        def _():
            def sl(g, carry2):
                slow_group(qb, g)
                return carry2
            lax.fori_loop(0, G, sl, 0)
            bad[...] = jnp.zeros(bad.shape, f32)

        slot = qb % 2
        oa = jnp.dot(woaT[...], ota[...].astype(bf16), preferred_element_type=f32)
        ob = jnp.dot(wobT[...], otb[...].astype(bf16), preferred_element_type=f32)
        o = jnp.concatenate([oa, ob], axis=0).astype(bf16)

        @pl.when(qb >= 2)
        def _():
            cp_out(qb - 2, slot).wait()
        obuf[slot] = o.T
        cp_out(qb, slot).start()
        return carry

    lax.fori_loop(0, NQB, qblock, 0)
    cp_out(NQB - 2, 0).wait()
    cp_out(NQB - 1, 1).wait()


@jax.jit
def pallas_concat_heads__sliding_block__grouped_kv_mqa__prompt_kernel(
    A_x, A_wqkv, A_wo, B_x, B_wq, B_wk, B_wv, B_wo
):
    scale = float(np.asarray(DH ** -0.5, dtype=A_x.dtype))
    scratch = [
        pltpu.VMEM((D, S), bf16),
        pltpu.VMEM((D, S), bf16),
        pltpu.VMEM((D, 3 * D), bf16),
        pltpu.VMEM((D, D), bf16),
        pltpu.VMEM((D, D), bf16),
        pltpu.VMEM((D, D), bf16),
        pltpu.VMEM((DH, D), bf16),
        pltpu.VMEM((DH, D), bf16),
        pltpu.VMEM((3 * D, D), bf16),
        pltpu.VMEM((D, D), bf16),
        pltpu.VMEM((D, D), bf16),
        pltpu.VMEM((D, D), bf16),
        pltpu.VMEM((D, S), f32),
        pltpu.VMEM((D, S), f32),
        pltpu.VMEM((G, WIN + S, 128), bf16),
        pltpu.VMEM((G, 4, 24, WIN + S), f32),
        pltpu.VMEM((S, 128), bf16),
        pltpu.VMEM((4, 24, S), f32),
        pltpu.VMEM((G + 1, 8, 128), f32),
        pltpu.VMEM((2, 24, QB), f32),
        pltpu.VMEM((D, QB), f32),
        pltpu.VMEM((D, QB), f32),
        pltpu.VMEM((8, QB), f32),
        pltpu.VMEM((2, QB, 2 * D), bf16),
        pltpu.SemaphoreType.DMA((2 * NQB + 6,)),
        pltpu.SemaphoreType.DMA((2,)),
    ]
    anyspec = pl.BlockSpec(memory_space=pl.ANY)
    out = pl.pallas_call(
        functools.partial(kernel, scale),
        out_shape=jax.ShapeDtypeStruct((S, 2 * D), A_x.dtype),
        in_specs=[anyspec] * 8,
        out_specs=anyspec,
        scratch_shapes=scratch,
        compiler_params=pltpu.CompilerParams(vmem_limit_bytes=100 * 1024 * 1024),
    )(A_x[0].T, A_wqkv, A_wo, B_x[0].T, B_wq, B_wk.T, B_wv.T, B_wo)
    return out[None]


run = pallas_concat_heads__sliding_block__grouped_kv_mqa__prompt_kernel
```

```python
import functools

import jax
import jax.numpy as jnp
import numpy as np
from jax import lax
from jax.experimental import pallas as pl
from jax.experimental.pallas import tpu as pltpu

S = 2048
D = 576
DH = 18
WIN = 256
G = 8
GU = 2
QB = 512
NQB = S // QB
NT = QB // 128
PB = 512
NPB = S // PB
KC = 256
NC = S // KC
APOS = (13, 20, 27, 30)
LOG2E = 1.4426950408889634
R0 = (0, 16, 32, 48)
OFF = (0, 2, 4, 6)
SHIFT = 64.0
LMIN = 2.0 ** -6
BIG = 3.0e38
f32 = jnp.float32
bf16 = jnp.bfloat16


def _rows(n, m):
    return lax.broadcasted_iota(jnp.int32, (n, m), 0)


def _lanes(n, m):
    return lax.broadcasted_iota(jnp.int32, (n, m), 1)


def _bf(x):
    return x.astype(bf16).astype(f32)


def _dot(a, b):
    return lax.dot_general(a, b, (((1,), (0,)), ((), ())), preferred_element_type=f32)


def _lrow(j):
    return (OFF[j] + DH) % 24


def _norm(acc, j):
    r = _lrow(j)
    return acc * (1.0 / acc[r:r + 1, :])


def _merge(n):
    row = _rows(8, n[0].shape[1])
    return jnp.concatenate([
        n[0][0:16],
        jnp.where(row < 2, n[0][16:24], n[1][0:8]),
        n[1][8:16],
        jnp.where(row < 4, n[1][16:24], n[2][0:8]),
        n[2][8:16],
        jnp.where(row < 6, n[2][16:24], n[3][0:8]),
        n[3][8:24],
    ], axis=0)


def _absbits_max(x):
    b = pltpu.bitcast(x, jnp.int32) & 0x7FFFFFFF
    r = None
    for i in range(x.shape[0] // 8):
        for t in range(x.shape[1] // 128):
            v = b[8 * i:8 * i + 8, 128 * t:128 * t + 128]
            r = v if r is None else jnp.maximum(r, v)
    return r


def _lmin(acc, j):
    l = acc[_lrow(j):_lrow(j) + 1, :]
    r = l[:, 0:128]
    for t in range(1, acc.shape[1] // 128):
        r = jnp.minimum(r, l[:, 128 * t:128 * t + 128])
    return r


def _kernel(scale, xa_hbm, wqkv_hbm, woa_hbm, xb_hbm, wq_hbm, wkT_hbm, wvT_hbm, wob_hbm, out_hbm,
            xa_v, xb_v, wqkv_v, wq_v, woa_v, wob_v, wkT_v, wvT_v,
            wqkvT, wqT, woaT, wobT, qta, qtb, kpa, va, kb, vb, kma, kv24, ota, otb,
            bad, lmin, accc, obuf, in_sem, out_sem):
    c = scale * LOG2E

    def cols(sb):
        return pl.ds(pl.multiple_of(sb * PB, PB), PB)

    def qcols(qb):
        return pl.ds(pl.multiple_of(qb * QB, QB), QB)

    def cp_xb(sb):
        return pltpu.make_async_copy(xb_hbm.at[:, cols(sb)], xb_v.at[:, cols(sb)], in_sem.at[sb])

    def cp_xa(sb):
        return pltpu.make_async_copy(xa_hbm.at[:, cols(sb)], xa_v.at[:, cols(sb)], in_sem.at[NPB + sb])

    cp_wq, cp_wk, cp_wv, cp_wqkv, cp_woa, cp_wob = [
        pltpu.make_async_copy(src, dst, in_sem.at[2 * NPB + i]) for i, (src, dst) in enumerate(
            [(wq_hbm, wq_v), (wkT_hbm, wkT_v), (wvT_hbm, wvT_v),
             (wqkv_hbm, wqkv_v), (woa_hbm, woa_v), (wob_hbm, wob_v)])]
    for cp in (cp_wq, cp_xb(0), cp_wk, cp_wv, cp_xb(1), cp_xb(2), cp_wqkv, cp_xb(3),
               cp_xa(0), cp_woa, cp_wob, cp_xa(1), cp_xa(2), cp_xa(3)):
        cp.start()

    kpa[:, 0:WIN, :] = jnp.zeros((G, WIN, 128), bf16)
    va[:, :, :, 0:WIN] = jnp.zeros((G, 4, 24, WIN), f32)
    kma[...] = jnp.zeros(kma.shape, f32)
    kv24[...] = jnp.zeros(kv24.shape, f32)
    bad[...] = jnp.zeros(bad.shape, jnp.int32)
    lmin[...] = jnp.full(lmin.shape, BIG, f32)
    accc[...] = jnp.ones(accc.shape, f32)
    row24 = _rows(24, PB)
    row24q = _rows(24, QB)

    def proj_b(sb):
        cs = cols(sb)
        xb = xb_v[:, cs]
        kv24[0, 0:DH, :] = _bf(_dot(wkT_v[...], xb))
        kv24[1, 0:DH, :] = _bf(_dot(wvT_v[...], xb))
        k24 = kv24[0]
        v24 = kv24[1]
        kaug = jnp.where(row24 == DH, 1.0, k24)
        kb[cs, :] = jnp.concatenate([kaug, jnp.zeros((104, PB), f32)], axis=0).astype(bf16).T
        n2 = jnp.max(jnp.sum(k24 * k24, axis=0, keepdims=True), axis=1, keepdims=True)
        kma[G, 0:1, :] = jnp.maximum(kma[G, 0:1, :], jnp.broadcast_to(n2, (1, 128)))
        v1 = jnp.where(row24 == DH, 1.0, v24)
        for j in range(4):
            vb[j, :, cs] = v1 if OFF[j] == 0 else pltpu.roll(v1, OFF[j], 0)
        qtb[:, cs] = _dot(wqT[...], xb) * c

    cp_wq.wait()
    cp_wk.wait()
    cp_wv.wait()
    cp_xb(0).wait()
    wqT[...] = wq_v[...].T
    proj_b(0)
    cp_xb(1).wait()
    cp_xb(2).wait()
    proj_b(1)
    proj_b(2)
    cp_wqkv.wait()
    cp_xb(3).wait()
    wqkvT[...] = wqkv_v[...].T
    proj_b(3)

    def proj_a(sb, extra=()):
        cp_xa(sb).wait()
        cs = cols(sb)
        csp = pl.ds(pl.multiple_of(sb * PB + WIN, 128), PB)
        xa = xa_v[:, cs]
        for e in extra:
            e()
        ka = _bf(_dot(wqkvT[D:2 * D, :], xa))
        one8 = jnp.where(_rows(8, PB) < 4, 1.0, 0.0).astype(f32)
        for g in range(G):
            kg = ka[72 * g:72 * g + 72]
            kpa[g, csp, :] = jnp.concatenate([kg, one8, jnp.zeros((48, PB), f32)], axis=0).astype(bf16).T
            sq = kg * kg
            for j in range(4):
                w = jnp.where((row24 >= OFF[j]) & (row24 < OFF[j] + DH), sq[R0[j]:R0[j] + 24], 0.0)
                n2 = jnp.max(jnp.sum(w, axis=0, keepdims=True), axis=1, keepdims=True)
                kma[g, j:j + 1, :] = jnp.maximum(kma[g, j:j + 1, :], jnp.broadcast_to(n2, (1, 128)))
        vaT = _bf(_dot(wqkvT[2 * D:3 * D, :], xa))
        for g in range(G):
            for j in range(4):
                r = 72 * g + R0[j]
                va[g, j, :, csp] = jnp.where(row24 == _lrow(j), 1.0, vaT[r:r + 24])
        qta[:, cs] = _dot(wqkvT[0:D, :], xa) * c

    def t_woa():
        woaT[...] = woa_v[...].T

    def t_wob():
        wobT[...] = wob_v[...].T

    cp_woa.wait()
    cp_wob.wait()
    proj_a(0, (t_woa, t_wob))

    def proj_a_loop(sb, carry):
        proj_a(sb)
        return carry

    lax.fori_loop(1, NPB, proj_a_loop, 0)

    rowhead = _rows(80, 128)
    rowhead = jnp.where(rowhead >= 72, rowhead - 72,
                        jnp.where(rowhead >= 54, 3, jnp.where(rowhead >= 36, 2, jnp.where(rowhead >= 18, 1, 0))))
    zsel = (((_lanes(80, 128) >> 6) - rowhead) & 1) + 2 * (rowhead >> 1)
    m_lo = _rows(64, 128) > (_lanes(64, 128) & 63)
    m_hi = _rows(64, 128) <= (_lanes(64, 128) & 63)
    lblk64 = _lanes(64, 128) >> 6

    def build_wa(qb, g, t):
        q = qta[pl.ds(pl.multiple_of(72 * g, 8), 72), pl.ds(pl.multiple_of(qb * QB + 128 * t, 128), 128)]
        sq = q * q
        r24 = _rows(24, 128)
        r8 = _rows(8, 128)
        mrow = jnp.zeros((8, 128), f32)
        for j in range(4):
            w = jnp.where((r24 >= OFF[j]) & (r24 < OFF[j] + DH), sq[R0[j]:R0[j] + 24], 0.0)
            m = jnp.sqrt(jnp.sum(w, axis=0, keepdims=True) * kma[g, j:j + 1, :]) * 1.01 - SHIFT
            mrow = jnp.where(r8 == j, -m, mrow)
        x = jnp.concatenate([q, mrow], axis=0)
        xr = jnp.where((rowhead & 1) == 1, pltpu.roll(x, 64, 1), x)
        z48 = jnp.zeros((48, 128), f32)
        return [jnp.concatenate([jnp.where(zsel == u, xr, 0.0), z48], axis=0).astype(bf16) for u in range(4)]

    def qb_win(qb, g, j):
        qwin = qtb[pl.ds(pl.multiple_of(72 * g + R0[j], 8), 24), qcols(qb)]
        if OFF[j]:
            qwin = pltpu.roll(qwin, 24 - OFF[j], 0)
        return jnp.where(row24q < DH, qwin, 0.0)

    def build_wb(qb, g, j):
        qm = qb_win(qb, g, j)
        km = jnp.concatenate([kma[G, 0:1, :]] * NT, axis=1)
        m = jnp.sqrt(jnp.sum(qm * qm, axis=0, keepdims=True) * km) * 1.01 - SHIFT
        qm = jnp.where(row24q == DH, -m, qm)
        return jnp.concatenate([qm, jnp.zeros((104, QB), f32)], axis=0).astype(bf16)

    def finish_b(g, j, acc):
        on = _norm(acc, j)
        keep = (row24q >= OFF[j]) & (row24q < OFF[j] + DH)
        pltpu.store(otb.at[pl.ds(pl.multiple_of(72 * g + R0[j], 8), 24), :], on, mask=keep)
        return _lmin(acc, j), _absbits_max(on)

    def flag(pairs):
        l, fin = pairs[0]
        for a, b in pairs[1:]:
            l, fin = jnp.minimum(l, a), jnp.maximum(fin, b)
        lmin[...] = jnp.minimum(lmin[...], l)
        bad[...] = jnp.maximum(bad[...], fin)

    def group(qb, g, u):
        q0 = pl.multiple_of(qb * QB, QB)
        rows = pl.ds(pl.multiple_of(72 * g, 8), 72)
        flags = []
        if u == 0:
            l, fin = finish_b((g + G - 1) % G, 3, accc[...])
            flags.append((jnp.where(g > 0, l, BIG), jnp.where(g > 0, fin, 0)))
        st = {}
        bsteps, asteps = [], []
        for j in range(4):
            for cc in range(NC):
                def qk(j=j, cc=cc):
                    if cc == 0:
                        st['wb', j] = build_wb(qb, g, j)
                    return _dot(kb[cc * KC:(cc + 1) * KC, :], st['wb', j])

                def post(s):
                    return jnp.exp2(s).astype(bf16)

                def pv(p, j=j, cc=cc):
                    o = _dot(vb[j, :, cc * KC:(cc + 1) * KC], p)
                    st['acc', j] = o if cc == 0 else st['acc', j] + o
                    if cc == NC - 1:
                        if j == 3 and u == GU - 1:
                            accc[...] = st['acc', j]
                        else:
                            flags.append(finish_b(g, j, st['acc', j]))
                bsteps.append((qk, post, pv))
        for t in range(NT):
            def qk(t=t):
                ws = build_wa(qb, g, t)
                k0 = q0 + 128 * t
                return [_dot(kpa[g, pl.ds(pl.multiple_of(k0 + 64 * (r & 1), 64), 320), :], ws[r])
                        for r in range(4)]

            def post(ss):
                es = []
                for r in range(4):
                    e = jnp.exp2(ss[r])
                    es.append([jnp.where(m_lo, e[0:64], 0.0), e[64:128], e[128:192], e[192:256],
                               jnp.where(m_hi, e[256:320], 0.0)])
                ps = []
                for h in range(4):
                    e0, e1 = es[2 * (h >> 1)], es[2 * (h >> 1) + 1]
                    m0 = lblk64 == (h & 1)
                    pieces = [jnp.where(m0, e0[0], 0.0)]
                    for a in range(1, 5):
                        pieces.append(jnp.where(m0, e0[a], e1[a - 1]))
                    pieces.append(jnp.where(m0, 0.0, e1[4]))
                    ps.append(jnp.concatenate(pieces, axis=0).astype(bf16))
                return ps

            def pv(p, t=t):
                k0 = pl.multiple_of(q0 + 128 * t, 128)
                o, lm = [], None
                for j in range(4):
                    acc = _dot(va[g, j, :, pl.ds(k0, 384)], p[j])
                    on = _norm(acc, j)
                    o.append(on if j % 2 == 0 else pltpu.roll(on, 64, 1))
                    lm = _lmin(acc, j) if lm is None else jnp.minimum(lm, _lmin(acc, j))
                blk = _merge(o)
                ota[rows, 128 * t:128 * t + 128] = blk
                flags.append((lm, _absbits_max(blk)))
            asteps.append((qk, post, pv))
        steps = []
        for i, b in enumerate(bsteps):
            steps += [a for a, pos in zip(asteps, APOS) if pos == i]
            steps.append(b)
        n = len(steps)
        ps, pend = {}, []
        for i in range(n):
            ps[i] = steps[i][1](steps[i][0]())
            pend.append(i)
            lag = 2 if i >= n - 2 else 1
            while pend and pend[0] <= i - lag:
                k = pend.pop(0)
                steps[k][2](ps[k])
        for k in pend:
            steps[k][2](ps[k])
        flag(flags)

    def slow_group(qb, g):
        q0 = qb * QB
        rows = pl.ds(pl.multiple_of(72 * g, 8), 72)
        nb, na = [], []
        for j in range(4):
            wb = jnp.concatenate([qb_win(qb, g, j), jnp.zeros((104, QB), f32)], axis=0).astype(bf16)

            def sb_(cc, wb=wb):
                return _dot(kb[pl.ds(pl.multiple_of(cc * KC, KC), KC), :], wb)

            m = lax.fori_loop(0, NC, lambda cc, m: jnp.maximum(m, jnp.max(sb_(cc), axis=0, keepdims=True)),
                              jnp.full((1, QB), -jnp.inf, f32))
            acc = lax.fori_loop(
                0, NC,
                lambda cc, a, j=j, m=m: a + _dot(vb[j, :, pl.ds(pl.multiple_of(cc * KC, KC), KC)],
                                                 jnp.exp2(sb_(cc) - m).astype(bf16)),
                jnp.zeros((24, QB), f32))
            nb.append(_norm(acc, j))

            qwin = qta[pl.ds(pl.multiple_of(72 * g + R0[j], 8), 24), qcols(qb)]
            qm = jnp.where((row24q >= OFF[j]) & (row24q < OFF[j] + DH), qwin, 0.0)
            parts = [jnp.zeros((R0[j], QB), f32)] if R0[j] else []
            parts += [qm, jnp.zeros((128 - R0[j] - 24, QB), f32)]
            wa = jnp.concatenate(parts, axis=0).astype(bf16)

            def sa_(cc, wa=wa):
                s = _dot(kpa[g, pl.ds(pl.multiple_of(cc * KC + WIN, KC), KC), :], wa)
                dist = (q0 - cc * KC) + _lanes(KC, QB) - _rows(KC, QB)
                return jnp.where((dist >= 0) & (dist < WIN), s, -1e9 * LOG2E)

            m = lax.fori_loop(0, NC, lambda cc, m: jnp.maximum(m, jnp.max(sa_(cc), axis=0, keepdims=True)),
                              jnp.full((1, QB), -jnp.inf, f32))
            acc = lax.fori_loop(
                0, NC,
                lambda cc, a, j=j, m=m: a + _dot(va[g, j, :, pl.ds(pl.multiple_of(cc * KC + WIN, KC), KC)],
                                                 jnp.exp2(sa_(cc) - m).astype(bf16)),
                jnp.zeros((24, QB), f32))
            na.append(_norm(acc, j))
        otb[rows, :] = _merge(nb)
        ota[rows, :] = _merge(na)

    def cp_out(qb, slot):
        return pltpu.make_async_copy(obuf.at[slot], out_hbm.at[pl.ds(pl.multiple_of(qb * QB, QB), QB), :],
                                     out_sem.at[slot])

    def qblock(qb, carry):
        def gl(i, carry2):
            for u in range(GU):
                group(qb, i * GU + u, u)
            return carry2

        lax.fori_loop(0, G // GU, gl, 0)
        flag([finish_b(G - 1, 3, accc[...])])

        unsafe = jnp.logical_or(jnp.max(bad[...]) >= 0x7F800000,
                                jnp.logical_not(jnp.min(lmin[...]) >= LMIN))

        @pl.when(unsafe)
        def _():
            def sl(g, carry2):
                slow_group(qb, g)
                return carry2

            lax.fori_loop(0, G, sl, 0)
            bad[...] = jnp.zeros(bad.shape, jnp.int32)
            lmin[...] = jnp.full(lmin.shape, BIG, f32)

        slot = qb % 2

        @pl.when(qb >= 2)
        def _():
            cp_out(qb - 2, slot).wait()

        oa = ota[...].astype(bf16)
        ob = otb[...].astype(bf16)
        for r in range(0, 2 * D, 128):
            if r + 128 <= D:
                o = _dot(woaT[r:r + 128, :], oa)
            elif r >= D:
                o = _dot(wobT[r - D:r - D + 128, :], ob)
            else:
                o = jnp.concatenate([_dot(woaT[r:D, :], oa), _dot(wobT[0:r + 128 - D, :], ob)], axis=0)
            obuf[slot, :, r:r + 128] = o.astype(bf16).T
        cp_out(qb, slot).start()
        return carry

    lax.fori_loop(0, NQB, qblock, 0)
    cp_out(NQB - 2, 0).wait()
    cp_out(NQB - 1, 1).wait()


@jax.jit
def pallas_concat_heads__sliding_block__grouped_kv_mqa__prompt_kernel(
    A_x: jax.Array,
    A_wqkv: jax.Array,
    A_wo: jax.Array,
    B_x: jax.Array,
    B_wq: jax.Array,
    B_wk: jax.Array,
    B_wv: jax.Array,
    B_wo: jax.Array,
):
    scale = float(np.asarray(DH ** -0.5, dtype=A_x.dtype))
    scratch = [
        pltpu.VMEM((D, S), bf16),
        pltpu.VMEM((D, S), bf16),
        pltpu.VMEM((D, 3 * D), bf16),
        pltpu.VMEM((D, D), bf16),
        pltpu.VMEM((D, D), bf16),
        pltpu.VMEM((D, D), bf16),
        pltpu.VMEM((DH, D), bf16),
        pltpu.VMEM((DH, D), bf16),
        pltpu.VMEM((3 * D, D), bf16),
        pltpu.VMEM((D, D), bf16),
        pltpu.VMEM((D, D), bf16),
        pltpu.VMEM((D, D), bf16),
        pltpu.VMEM((D, S), f32),
        pltpu.VMEM((D, S), f32),
        pltpu.VMEM((G, WIN + S, 128), bf16),
        pltpu.VMEM((G, 4, 24, WIN + S), f32),
        pltpu.VMEM((S, 128), bf16),
        pltpu.VMEM((4, 24, S), f32),
        pltpu.VMEM((G + 1, 8, 128), f32),
        pltpu.VMEM((2, 24, PB), f32),
        pltpu.VMEM((D, QB), f32),
        pltpu.VMEM((D, QB), f32),
        pltpu.VMEM((8, 128), jnp.int32),
        pltpu.VMEM((1, 128), f32),
        pltpu.VMEM((24, QB), f32),
        pltpu.VMEM((2, QB, 2 * D), bf16),
        pltpu.SemaphoreType.DMA((2 * NPB + 6,)),
        pltpu.SemaphoreType.DMA((2,)),
    ]
    anyspec = pl.BlockSpec(memory_space=pl.ANY)
    out = pl.pallas_call(
        functools.partial(_kernel, scale),
        out_shape=jax.ShapeDtypeStruct((S, 2 * D), A_x.dtype),
        in_specs=[anyspec] * 8,
        out_specs=anyspec,
        scratch_shapes=scratch,
        compiler_params=pltpu.CompilerParams(vmem_limit_bytes=100 * 1024 * 1024),
    )(A_x[0].T, A_wqkv, A_wo, B_x[0].T, B_wq, B_wk.T, B_wv.T, B_wo)
    return out[None]
```

```python
import functools

import jax
import jax.numpy as jnp
import numpy as np
from jax import lax
from jax.experimental import pallas as pl
from jax.experimental.pallas import tpu as pltpu

S = 2048
D = 576
DH = 18
WIN = 256
G = 8
GU = 2
QB = 512
NQB = S // QB
NT = QB // 128
PB = 512
NPB = S // PB
KC = 256
NC = S // KC
APOS = (13, 20, 27, 30)
LOG2E = 1.4426950408889634
R0 = (0, 16, 32, 48)
OFF = (0, 2, 4, 6)
SHIFT = 64.0
LMIN = 2.0 ** -6
BIG = 3.0e38
f32 = jnp.float32
bf16 = jnp.bfloat16


def _rows(n, m):
    return lax.broadcasted_iota(jnp.int32, (n, m), 0)


def _lanes(n, m):
    return lax.broadcasted_iota(jnp.int32, (n, m), 1)


def _bf(x):
    return x.astype(bf16).astype(f32)


def _dot(a, b):
    return lax.dot_general(a, b, (((1,), (0,)), ((), ())), preferred_element_type=f32)


def _lrow(j):
    return (OFF[j] + DH) % 24


def _norm(acc, j):
    r = _lrow(j)
    return acc * (1.0 / acc[r:r + 1, :])


def _merge(n):
    row = _rows(8, n[0].shape[1])
    return jnp.concatenate([
        n[0][0:16],
        jnp.where(row < 2, n[0][16:24], n[1][0:8]),
        n[1][8:16],
        jnp.where(row < 4, n[1][16:24], n[2][0:8]),
        n[2][8:16],
        jnp.where(row < 6, n[2][16:24], n[3][0:8]),
        n[3][8:24],
    ], axis=0)


def _absbits_max(x):
    b = pltpu.bitcast(x, jnp.int32) & 0x7FFFFFFF
    r = None
    for i in range(x.shape[0] // 8):
        for t in range(x.shape[1] // 128):
            v = b[8 * i:8 * i + 8, 128 * t:128 * t + 128]
            r = v if r is None else jnp.maximum(r, v)
    return r


def _lmin(acc, j):
    l = acc[_lrow(j):_lrow(j) + 1, :]
    r = l[:, 0:128]
    for t in range(1, acc.shape[1] // 128):
        r = jnp.minimum(r, l[:, 128 * t:128 * t + 128])
    return r


def _kernel(scale, xa_hbm, wqkv_hbm, woa_hbm, xb_hbm, wq_hbm, wkT_hbm, wvT_hbm, wob_hbm, out_hbm,
            xa_v, xb_v, wqkv_v, wq_v, woa_v, wob_v, wkT_v, wvT_v,
            wqkvT, wqT, woT, qta, qtb, kpa, va, kb, vb, kma, kv24, ota, otb,
            bad, lmin, accc, obuf, in_sem, out_sem):
    c = scale * LOG2E

    def cols(sb):
        return pl.ds(pl.multiple_of(sb * PB, PB), PB)

    def qcols(qb):
        return pl.ds(pl.multiple_of(qb * QB, QB), QB)

    def cp_xb(sb):
        return pltpu.make_async_copy(xb_hbm.at[:, cols(sb)], xb_v.at[:, cols(sb)], in_sem.at[sb])

    def cp_xa(sb):
        return pltpu.make_async_copy(xa_hbm.at[:, cols(sb)], xa_v.at[:, cols(sb)], in_sem.at[NPB + sb])

    cp_wq, cp_wk, cp_wv, cp_wqkv, cp_woa, cp_wob = [
        pltpu.make_async_copy(src, dst, in_sem.at[2 * NPB + i]) for i, (src, dst) in enumerate(
            [(wq_hbm, wq_v), (wkT_hbm, wkT_v), (wvT_hbm, wvT_v),
             (wqkv_hbm, wqkv_v), (woa_hbm, woa_v), (wob_hbm, wob_v)])]
    for cp in (cp_wq, cp_xb(0), cp_wk, cp_wv, cp_xb(1), cp_xb(2), cp_wqkv, cp_xb(3),
               cp_xa(0), cp_woa, cp_wob, cp_xa(1), cp_xa(2), cp_xa(3)):
        cp.start()

    kpa[:, 0:WIN, :] = jnp.zeros((G, WIN, 128), bf16)
    va[:, :, :, 0:WIN] = jnp.zeros((G, 4, 24, WIN), f32)
    kma[...] = jnp.zeros(kma.shape, f32)
    kv24[...] = jnp.zeros(kv24.shape, f32)
    bad[...] = jnp.zeros(bad.shape, jnp.int32)
    lmin[...] = jnp.full(lmin.shape, BIG, f32)
    accc[...] = jnp.ones(accc.shape, f32)
    row24 = _rows(24, PB)
    row24q = _rows(24, QB)

    def proj_b(sb):
        cs = cols(sb)
        xb = xb_v[:, cs]
        kv24[0, 0:DH, :] = _bf(_dot(wkT_v[...], xb))
        kv24[1, 0:DH, :] = _bf(_dot(wvT_v[...], xb))
        k24 = kv24[0]
        v24 = kv24[1]
        kaug = jnp.where(row24 == DH, 1.0, k24)
        kb[cs, :] = jnp.concatenate([kaug, jnp.zeros((104, PB), f32)], axis=0).astype(bf16).T
        n2 = jnp.max(jnp.sum(k24 * k24, axis=0, keepdims=True), axis=1, keepdims=True)
        kma[G, 0:1, :] = jnp.maximum(kma[G, 0:1, :], jnp.broadcast_to(n2, (1, 128)))
        v1 = jnp.where(row24 == DH, 1.0, v24)
        for j in range(4):
            vb[j, :, cs] = v1 if OFF[j] == 0 else pltpu.roll(v1, OFF[j], 0)
        qtb[:, cs] = _dot(wqT[...], xb) * c

    cp_wq.wait()
    cp_wk.wait()
    cp_wv.wait()
    cp_xb(0).wait()
    wqT[...] = wq_v[...].T
    proj_b(0)
    cp_xb(1).wait()
    cp_xb(2).wait()
    proj_b(1)
    proj_b(2)
    cp_wqkv.wait()
    cp_xb(3).wait()
    wqkvT[...] = wqkv_v[...].T
    proj_b(3)

    def proj_a(sb, extra=()):
        cp_xa(sb).wait()
        cs = cols(sb)
        csp = pl.ds(pl.multiple_of(sb * PB + WIN, 128), PB)
        xa = xa_v[:, cs]
        for e in extra:
            e()
        ka = _bf(_dot(wqkvT[D:2 * D, :], xa))
        one8 = jnp.where(_rows(8, PB) < 4, 1.0, 0.0).astype(f32)
        for g in range(G):
            kg = ka[72 * g:72 * g + 72]
            kpa[g, csp, :] = jnp.concatenate([kg, one8, jnp.zeros((48, PB), f32)], axis=0).astype(bf16).T
            sq = kg * kg
            for j in range(4):
                w = jnp.where((row24 >= OFF[j]) & (row24 < OFF[j] + DH), sq[R0[j]:R0[j] + 24], 0.0)
                n2 = jnp.max(jnp.sum(w, axis=0, keepdims=True), axis=1, keepdims=True)
                kma[g, j:j + 1, :] = jnp.maximum(kma[g, j:j + 1, :], jnp.broadcast_to(n2, (1, 128)))
        vaT = _bf(_dot(wqkvT[2 * D:3 * D, :], xa))
        for g in range(G):
            for j in range(4):
                r = 72 * g + R0[j]
                va[g, j, :, csp] = jnp.where(row24 == _lrow(j), 1.0, vaT[r:r + 24])
        qta[:, cs] = _dot(wqkvT[0:D, :], xa) * c

    def t_woa():
        woT[0:D] = woa_v[...].T

    def t_wob():
        woT[D:2 * D] = wob_v[...].T

    cp_woa.wait()
    cp_wob.wait()
    proj_a(0, (t_woa, t_wob))

    def proj_a_loop(sb, carry):
        proj_a(sb)
        return carry

    lax.fori_loop(1, NPB, proj_a_loop, 0)

    rowhead = _rows(80, 128)
    rowhead = jnp.where(rowhead >= 72, rowhead - 72,
                        jnp.where(rowhead >= 54, 3, jnp.where(rowhead >= 36, 2, jnp.where(rowhead >= 18, 1, 0))))
    zsel = (((_lanes(80, 128) >> 6) - rowhead) & 1) + 2 * (rowhead >> 1)
    m_lo = _rows(64, 128) > (_lanes(64, 128) & 63)
    m_hi = _rows(64, 128) <= (_lanes(64, 128) & 63)
    lblk64 = _lanes(64, 128) >> 6

    def build_wa(qb, g, t):
        q = qta[pl.ds(pl.multiple_of(72 * g, 8), 72), pl.ds(pl.multiple_of(qb * QB + 128 * t, 128), 128)]
        sq = q * q
        r24 = _rows(24, 128)
        r8 = _rows(8, 128)
        mrow = jnp.zeros((8, 128), f32)
        for j in range(4):
            w = jnp.where((r24 >= OFF[j]) & (r24 < OFF[j] + DH), sq[R0[j]:R0[j] + 24], 0.0)
            m = jnp.sqrt(jnp.sum(w, axis=0, keepdims=True) * kma[g, j:j + 1, :]) * 1.01 - SHIFT
            mrow = jnp.where(r8 == j, -m, mrow)
        x = jnp.concatenate([q, mrow], axis=0)
        xr = jnp.where((rowhead & 1) == 1, pltpu.roll(x, 64, 1), x)
        z48 = jnp.zeros((48, 128), f32)
        return [jnp.concatenate([jnp.where(zsel == u, xr, 0.0), z48], axis=0).astype(bf16) for u in range(4)]

    def qb_win(qb, g, j):
        qwin = qtb[pl.ds(pl.multiple_of(72 * g + R0[j], 8), 24), qcols(qb)]
        if OFF[j]:
            qwin = pltpu.roll(qwin, 24 - OFF[j], 0)
        return jnp.where(row24q < DH, qwin, 0.0)

    def build_wb(qb, g, j):
        qm = qb_win(qb, g, j)
        km = jnp.concatenate([kma[G, 0:1, :]] * NT, axis=1)
        m = jnp.sqrt(jnp.sum(qm * qm, axis=0, keepdims=True) * km) * 1.01 - SHIFT
        qm = jnp.where(row24q == DH, -m, qm)
        return jnp.concatenate([qm, jnp.zeros((104, QB), f32)], axis=0).astype(bf16)

    def finish_b(g, j, acc):
        on = _norm(acc, j)
        keep = (row24q >= OFF[j]) & (row24q < OFF[j] + DH)
        pltpu.store(otb.at[pl.ds(pl.multiple_of(72 * g + R0[j], 8), 24), :], on, mask=keep)
        return _lmin(acc, j), _absbits_max(on)

    def flag(pairs):
        l, fin = pairs[0]
        for a, b in pairs[1:]:
            l, fin = jnp.minimum(l, a), jnp.maximum(fin, b)
        lmin[...] = jnp.minimum(lmin[...], l)
        bad[...] = jnp.maximum(bad[...], fin)

    def group(qb, g, u):
        q0 = pl.multiple_of(qb * QB, QB)
        rows = pl.ds(pl.multiple_of(72 * g, 8), 72)
        flags = []
        if u == 0:
            l, fin = finish_b((g + G - 1) % G, 3, accc[...])
            flags.append((jnp.where(g > 0, l, BIG), jnp.where(g > 0, fin, 0)))
        st = {}
        bsteps, asteps = [], []
        for j in range(4):
            for cc in range(NC):
                def qk(j=j, cc=cc):
                    if cc == 0:
                        st['wb', j] = build_wb(qb, g, j)
                    return _dot(kb[cc * KC:(cc + 1) * KC, :], st['wb', j])

                def post(s):
                    return jnp.exp2(s).astype(bf16)

                def pv(p, j=j, cc=cc):
                    o = _dot(vb[j, :, cc * KC:(cc + 1) * KC], p)
                    st['acc', j] = o if cc == 0 else st['acc', j] + o
                    if cc == NC - 1:
                        if j == 3 and u == GU - 1:
                            accc[...] = st['acc', j]
                        else:
                            flags.append(finish_b(g, j, st['acc', j]))
                bsteps.append((qk, post, pv))
        for t in range(NT):
            def qk(t=t):
                ws = build_wa(qb, g, t)
                k0 = q0 + 128 * t
                return [_dot(kpa[g, pl.ds(pl.multiple_of(k0 + 64 * (r & 1), 64), 320), :], ws[r])
                        for r in range(4)]

            def post(ss):
                es = []
                for r in range(4):
                    e = jnp.exp2(ss[r])
                    es.append([jnp.where(m_lo, e[0:64], 0.0), e[64:128], e[128:192], e[192:256],
                               jnp.where(m_hi, e[256:320], 0.0)])
                ps = []
                for h in range(4):
                    e0, e1 = es[2 * (h >> 1)], es[2 * (h >> 1) + 1]
                    m0 = lblk64 == (h & 1)
                    pieces = [jnp.where(m0, e0[0], 0.0)]
                    for a in range(1, 5):
                        pieces.append(jnp.where(m0, e0[a], e1[a - 1]))
                    pieces.append(jnp.where(m0, 0.0, e1[4]))
                    ps.append(jnp.concatenate(pieces, axis=0).astype(bf16))
                return ps

            def pv(p, t=t):
                k0 = pl.multiple_of(q0 + 128 * t, 128)
                o, lm = [], None
                for j in range(4):
                    acc = _dot(va[g, j, :, pl.ds(k0, 384)], p[j])
                    on = _norm(acc, j)
                    o.append(on if j % 2 == 0 else pltpu.roll(on, 64, 1))
                    lm = _lmin(acc, j) if lm is None else jnp.minimum(lm, _lmin(acc, j))
                blk = _merge(o)
                ota[rows, 128 * t:128 * t + 128] = blk
                flags.append((lm, _absbits_max(blk)))
            asteps.append((qk, post, pv))
        steps = []
        for i, b in enumerate(bsteps):
            steps += [a for a, pos in zip(asteps, APOS) if pos == i]
            steps.append(b)
        n = len(steps)
        ps, pend = {}, []
        for i in range(n):
            ps[i] = steps[i][1](steps[i][0]())
            pend.append(i)
            lag = 2 if i >= n - 2 else 1
            while pend and pend[0] <= i - lag:
                k = pend.pop(0)
                steps[k][2](ps[k])
        for k in pend:
            steps[k][2](ps[k])
        flag(flags)

    def slow_head(qb, h):
        g, j = h // 4, h % 4
        q0 = qb * QB
        off = 2 * j
        win = pl.ds(pl.multiple_of(72 * g + 16 * j, 8), 24)
        keep = (row24q >= off) & (row24q < off + DH)
        isl = row24q == (off + DH) % 24

        def attend(scores, values, dst):
            m = lax.fori_loop(0, NC, lambda cc, m: jnp.maximum(m, jnp.max(scores(cc), axis=0, keepdims=True)),
                              jnp.full((1, QB), -jnp.inf, f32))
            acc = lax.fori_loop(0, NC, lambda cc, a: a + _dot(values(cc), jnp.exp2(scores(cc) - m).astype(bf16)),
                                jnp.zeros((24, QB), f32))
            l = jnp.sum(jnp.where(isl, acc, 0.0), axis=0, keepdims=True)
            pltpu.store(dst.at[win, :], acc * (1.0 / l), mask=keep)

        qw = pltpu.roll(qtb[win, qcols(qb)], (24 - off) % 24, 0)
        wb = jnp.concatenate([jnp.where(row24q < DH, qw, 0.0), jnp.zeros((104, QB), f32)], axis=0).astype(bf16)
        attend(lambda cc: _dot(kb[pl.ds(pl.multiple_of(cc * KC, KC), KC), :], wb),
               lambda cc: vb[j, :, pl.ds(pl.multiple_of(cc * KC, KC), KC)], otb)

        r128 = _rows(128, QB)
        qg = jnp.concatenate([qta[pl.ds(pl.multiple_of(72 * g, 8), 72), qcols(qb)], jnp.zeros((56, QB), f32)], axis=0)
        wa = jnp.where((r128 >= DH * j) & (r128 < DH * j + DH), qg, 0.0).astype(bf16)

        def scores_a(cc):
            s = _dot(kpa[g, pl.ds(pl.multiple_of(cc * KC + WIN, KC), KC), :], wa)
            dist = (q0 - cc * KC) + _lanes(KC, QB) - _rows(KC, QB)
            return jnp.where((dist >= 0) & (dist < WIN), s, -1e9 * LOG2E)

        attend(scores_a, lambda cc: va[g, j, :, pl.ds(pl.multiple_of(cc * KC + WIN, KC), KC)], ota)

    def slow_out_proj(qb, slot):
        def chunk(i, carry):
            w = woT[pl.ds(pl.multiple_of(128 * i, 128), 128), :]
            o = jnp.where(_rows(128, QB) + 128 * i < D, _dot(w, ota[...].astype(bf16)), _dot(w, otb[...].astype(bf16)))
            obuf[slot, :, pl.ds(pl.multiple_of(128 * i, 128), 128)] = o.astype(bf16).T
            return carry

        lax.fori_loop(0, 2 * D // 128, chunk, 0)
        cp_out(qb, slot).start()

    def cp_out(qb, slot):
        return pltpu.make_async_copy(obuf.at[slot], out_hbm.at[pl.ds(pl.multiple_of(qb * QB, QB), QB), :],
                                     out_sem.at[slot])

    def out_proj(qb, slot):
        oa = ota[...].astype(bf16)
        ob = otb[...].astype(bf16)
        for r in range(0, 2 * D, 128):
            if r + 128 <= D:
                o = _dot(woT[r:r + 128, :], oa)
            elif r >= D:
                o = _dot(woT[r:r + 128, :], ob)
            else:
                o = jnp.concatenate([_dot(woT[r:D, :], oa), _dot(woT[D:r + 128, :], ob)], axis=0)
            obuf[slot, :, r:r + 128] = o.astype(bf16).T
        cp_out(qb, slot).start()

    def qblock(qb, carry):
        slot = qb % 2

        @pl.when(qb >= 2)
        def _():
            cp_out(qb - 2, slot).wait()

        def gl(i, carry2):
            for u in range(GU):
                group(qb, i * GU + u, u)
            return carry2

        lax.fori_loop(0, G // GU, gl, 0)
        flag([finish_b(G - 1, 3, accc[...])])
        out_proj(qb, slot)

        unsafe = jnp.logical_or(jnp.max(bad[...]) >= 0x7F800000,
                                jnp.logical_not(jnp.min(lmin[...]) >= LMIN))

        @pl.when(unsafe)
        def _():
            cp_out(qb, slot).wait()

            def sl(h, carry2):
                slow_head(qb, h)
                return carry2

            lax.fori_loop(0, 4 * G, sl, 0)
            bad[...] = jnp.zeros(bad.shape, jnp.int32)
            lmin[...] = jnp.full(lmin.shape, BIG, f32)
            slow_out_proj(qb, slot)

        return carry

    lax.fori_loop(0, NQB, qblock, 0)
    cp_out(NQB - 2, 0).wait()
    cp_out(NQB - 1, 1).wait()


@jax.jit
def pallas_concat_heads__sliding_block__grouped_kv_mqa__prompt_kernel(
    A_x: jax.Array,
    A_wqkv: jax.Array,
    A_wo: jax.Array,
    B_x: jax.Array,
    B_wq: jax.Array,
    B_wk: jax.Array,
    B_wv: jax.Array,
    B_wo: jax.Array,
):
    scale = float(np.asarray(DH ** -0.5, dtype=A_x.dtype))
    scratch = [
        pltpu.VMEM((D, S), bf16),
        pltpu.VMEM((D, S), bf16),
        pltpu.VMEM((D, 3 * D), bf16),
        pltpu.VMEM((D, D), bf16),
        pltpu.VMEM((D, D), bf16),
        pltpu.VMEM((D, D), bf16),
        pltpu.VMEM((DH, D), bf16),
        pltpu.VMEM((DH, D), bf16),
        pltpu.VMEM((3 * D, D), bf16),
        pltpu.VMEM((D, D), bf16),
        pltpu.VMEM((2 * D, D), bf16),
        pltpu.VMEM((D, S), f32),
        pltpu.VMEM((D, S), f32),
        pltpu.VMEM((G, WIN + S, 128), bf16),
        pltpu.VMEM((G, 4, 24, WIN + S), f32),
        pltpu.VMEM((S, 128), bf16),
        pltpu.VMEM((4, 24, S), f32),
        pltpu.VMEM((G + 1, 8, 128), f32),
        pltpu.VMEM((2, 24, PB), f32),
        pltpu.VMEM((D, QB), f32),
        pltpu.VMEM((D, QB), f32),
        pltpu.VMEM((8, 128), jnp.int32),
        pltpu.VMEM((1, 128), f32),
        pltpu.VMEM((24, QB), f32),
        pltpu.VMEM((2, QB, 2 * D), bf16),
        pltpu.SemaphoreType.DMA((2 * NPB + 6,)),
        pltpu.SemaphoreType.DMA((2,)),
    ]
    anyspec = pl.BlockSpec(memory_space=pl.ANY)
    out = pl.pallas_call(
        functools.partial(_kernel, scale),
        out_shape=jax.ShapeDtypeStruct((S, 2 * D), A_x.dtype),
        in_specs=[anyspec] * 8,
        out_specs=anyspec,
        scratch_shapes=scratch,
        compiler_params=pltpu.CompilerParams(vmem_limit_bytes=100 * 1024 * 1024),
    )(A_x[0].T, A_wqkv, A_wo, B_x[0].T, B_wq, B_wk.T, B_wv.T, B_wo)
    return out[None]
```

```python
import functools

import jax
import jax.numpy as jnp
import numpy as np
from jax import lax
from jax.experimental import pallas as pl
from jax.experimental.pallas import tpu as pltpu

S = 2048
D = 576
DH = 18
WIN = 256
G = 8
GU = 2
QB = 512
NQB = S // QB
NT = QB // 128
PB = 512
NPB = S // PB
KC = 256
NC = S // KC
APOS = (13, 20, 27, 30)
LOG2E = 1.4426950408889634
R0 = (0, 16, 32, 48)
OFF = (0, 2, 4, 6)
SHIFT = 64.0
LMIN = 2.0 ** -6
BIG = 3.0e38
f32 = jnp.float32
bf16 = jnp.bfloat16


def _rows(n, m):
    return lax.broadcasted_iota(jnp.int32, (n, m), 0)


def _lanes(n, m):
    return lax.broadcasted_iota(jnp.int32, (n, m), 1)


def _bf(x):
    return x.astype(bf16).astype(f32)


def _sqrt(x):
    return jnp.exp2(0.5 * jnp.log2(x))


def _dot(a, b):
    return lax.dot_general(a, b, (((1,), (0,)), ((), ())), preferred_element_type=f32)


def _lrow(j):
    return (OFF[j] + DH) % 24


def _norm(acc, j):
    r = _lrow(j)
    return acc * (1.0 / acc[r:r + 1, :])


def _merge(n):
    row = _rows(8, n[0].shape[1])
    return jnp.concatenate([
        n[0][0:16],
        jnp.where(row < 2, n[0][16:24], n[1][0:8]),
        n[1][8:16],
        jnp.where(row < 4, n[1][16:24], n[2][0:8]),
        n[2][8:16],
        jnp.where(row < 6, n[2][16:24], n[3][0:8]),
        n[3][8:24],
    ], axis=0)


def _absbits_max(x):
    b = pltpu.bitcast(x, jnp.int32) & 0x7FFFFFFF
    r = None
    for i in range(x.shape[0] // 8):
        for t in range(x.shape[1] // 128):
            v = b[8 * i:8 * i + 8, 128 * t:128 * t + 128]
            r = v if r is None else jnp.maximum(r, v)
    return r


def _lmin(acc, j):
    l = acc[_lrow(j):_lrow(j) + 1, :]
    r = l[:, 0:128]
    for t in range(1, acc.shape[1] // 128):
        r = jnp.minimum(r, l[:, 128 * t:128 * t + 128])
    return r


def _kernel(scale, xa_hbm, wqkv_hbm, woa_hbm, xb_hbm, wq_hbm, wkT_hbm, wvT_hbm, wob_hbm, out_hbm,
            xa_v, xb_v, wqkv_v, wq_v, woa_v, wob_v, wkT_v, wvT_v,
            wqkvT, wqT, woT, qta, qtb, kpa, va, kb, vb, kma, qna, qnb, kv24, ota, otb,
            bad, lmin, accc, obuf, in_sem, out_sem):
    c = scale * LOG2E

    def cols(sb):
        return pl.ds(pl.multiple_of(sb * PB, PB), PB)

    def qcols(qb):
        return pl.ds(pl.multiple_of(qb * QB, QB), QB)

    def cp_xb(sb):
        return pltpu.make_async_copy(xb_hbm.at[:, cols(sb)], xb_v.at[:, cols(sb)], in_sem.at[sb])

    def cp_xa(sb):
        return pltpu.make_async_copy(xa_hbm.at[:, cols(sb)], xa_v.at[:, cols(sb)], in_sem.at[NPB + sb])

    cp_wq, cp_wk, cp_wv, cp_wqkv, cp_woa, cp_wob = [
        pltpu.make_async_copy(src, dst, in_sem.at[2 * NPB + i]) for i, (src, dst) in enumerate(
            [(wq_hbm, wq_v), (wkT_hbm, wkT_v), (wvT_hbm, wvT_v),
             (wqkv_hbm, wqkv_v), (woa_hbm, woa_v), (wob_hbm, wob_v)])]
    for cp in (cp_wq, cp_xb(0), cp_wk, cp_wv, cp_xb(1), cp_xb(2), cp_wqkv, cp_xb(3),
               cp_xa(0), cp_woa, cp_wob, cp_xa(1), cp_xa(2), cp_xa(3)):
        cp.start()

    kpa[:, 0:WIN, :] = jnp.zeros((G, WIN, 128), bf16)
    va[:, :, :, 0:WIN] = jnp.zeros((G, 4, 24, WIN), f32)
    kma[...] = jnp.zeros(kma.shape, f32)
    kv24[...] = jnp.zeros(kv24.shape, f32)
    bad[...] = jnp.zeros(bad.shape, jnp.int32)
    lmin[...] = jnp.full(lmin.shape, BIG, f32)
    accc[...] = jnp.ones(accc.shape, f32)
    row24 = _rows(24, PB)
    row24q = _rows(24, QB)

    def store_q(q, q_ref, qn_ref, cs):
        q_ref[:, cs] = q
        sq = q * q
        for g in range(G):
            rows = []
            for j in range(4):
                r = 72 * g + R0[j]
                w = jnp.where((row24 >= OFF[j]) & (row24 < OFF[j] + DH), sq[r:r + 24], 0.0)
                rows.append(jnp.sum(w, axis=0, keepdims=True))
            r8 = _rows(8, PB)
            n2 = jnp.where(r8 == 0, rows[0], jnp.where(r8 == 1, rows[1], jnp.where(r8 == 2, rows[2], rows[3])))
            qn_ref[g, :, cs] = _sqrt(n2)

    def proj_b(sb):
        cs = cols(sb)
        xb = xb_v[:, cs]
        kv24[0, 0:DH, :] = _bf(_dot(wkT_v[...], xb))
        kv24[1, 0:DH, :] = _bf(_dot(wvT_v[...], xb))
        k24 = kv24[0]
        v24 = kv24[1]
        kaug = jnp.where(row24 == DH, 1.0, k24)
        kb[cs, :] = jnp.concatenate([kaug, jnp.zeros((104, PB), f32)], axis=0).astype(bf16).T
        n2 = jnp.max(jnp.sum(k24 * k24, axis=0, keepdims=True), axis=1, keepdims=True)
        kma[G, 0:1, :] = jnp.maximum(kma[G, 0:1, :], jnp.broadcast_to(n2, (1, 128)))
        v1 = jnp.where(row24 == DH, 1.0, v24)
        for j in range(4):
            vb[j, :, cs] = v1 if OFF[j] == 0 else pltpu.roll(v1, OFF[j], 0)
        store_q(_dot(wqT[...], xb) * c, qtb, qnb, cs)

    cp_wq.wait()
    cp_wk.wait()
    cp_wv.wait()
    cp_xb(0).wait()
    wqT[...] = wq_v[...].T
    proj_b(0)
    cp_xb(1).wait()
    cp_xb(2).wait()
    proj_b(1)
    proj_b(2)
    cp_wqkv.wait()
    cp_xb(3).wait()
    wqkvT[...] = wqkv_v[...].T
    proj_b(3)

    def proj_a(sb, extra=()):
        cp_xa(sb).wait()
        cs = cols(sb)
        csp = pl.ds(pl.multiple_of(sb * PB + WIN, 128), PB)
        xa = xa_v[:, cs]
        for e in extra:
            e()
        ka = _bf(_dot(wqkvT[D:2 * D, :], xa))
        one8 = jnp.where(_rows(8, PB) < 4, 1.0, 0.0).astype(f32)
        for g in range(G):
            kg = ka[72 * g:72 * g + 72]
            kpa[g, csp, :] = jnp.concatenate([kg, one8, jnp.zeros((48, PB), f32)], axis=0).astype(bf16).T
            sq = kg * kg
            for j in range(4):
                w = jnp.where((row24 >= OFF[j]) & (row24 < OFF[j] + DH), sq[R0[j]:R0[j] + 24], 0.0)
                n2 = jnp.max(jnp.sum(w, axis=0, keepdims=True), axis=1, keepdims=True)
                kma[g, j:j + 1, :] = jnp.maximum(kma[g, j:j + 1, :], jnp.broadcast_to(n2, (1, 128)))
        vaT = _bf(_dot(wqkvT[2 * D:3 * D, :], xa))
        for g in range(G):
            for j in range(4):
                r = 72 * g + R0[j]
                va[g, j, :, csp] = jnp.where(row24 == _lrow(j), 1.0, vaT[r:r + 24])
        store_q(_dot(wqkvT[0:D, :], xa) * c, qta, qna, cs)

    def t_woa():
        woT[0:D] = woa_v[...].T

    def t_wob():
        woT[D:2 * D] = wob_v[...].T

    cp_woa.wait()
    cp_wob.wait()
    proj_a(0, (t_woa, t_wob))

    def proj_a_loop(sb, carry):
        proj_a(sb)
        return carry

    lax.fori_loop(1, NPB, proj_a_loop, 0)

    kma[...] = _sqrt(kma[...]) * 1.01
    rowhead = _rows(80, 128)
    rowhead = jnp.where(rowhead >= 72, rowhead - 72,
                        jnp.where(rowhead >= 54, 3, jnp.where(rowhead >= 36, 2, jnp.where(rowhead >= 18, 1, 0))))
    zsel = (((_lanes(80, 128) >> 6) - rowhead) & 1) + 2 * (rowhead >> 1)
    m_lo = _rows(64, 128) > (_lanes(64, 128) & 63)
    m_hi = _rows(64, 128) <= (_lanes(64, 128) & 63)
    lblk64 = _lanes(64, 128) >> 6

    def build_wa(qb, g, t):
        q = qta[pl.ds(pl.multiple_of(72 * g, 8), 72), pl.ds(pl.multiple_of(qb * QB + 128 * t, 128), 128)]
        r8 = _rows(8, 128)
        qn = qna[g, :, pl.ds(pl.multiple_of(qb * QB + 128 * t, 128), 128)]
        mrow = jnp.where(r8 < 4, SHIFT - qn * kma[g], 0.0)
        x = jnp.concatenate([q, mrow], axis=0)
        xr = jnp.where((rowhead & 1) == 1, pltpu.roll(x, 64, 1), x)
        z48 = jnp.zeros((48, 128), f32)
        return [jnp.concatenate([jnp.where(zsel == u, xr, 0.0), z48], axis=0).astype(bf16) for u in range(4)]

    def qb_win(qb, g, j):
        qwin = qtb[pl.ds(pl.multiple_of(72 * g + R0[j], 8), 24), qcols(qb)]
        if OFF[j]:
            qwin = pltpu.roll(qwin, 24 - OFF[j], 0)
        return jnp.where(row24q < DH, qwin, 0.0)

    def build_wb(qb, g, j):
        qm = qb_win(qb, g, j)
        km = jnp.concatenate([kma[G, 0:1, :]] * NT, axis=1)
        m = qnb[g, j:j + 1, qcols(qb)] * km - SHIFT
        qm = jnp.where(row24q == DH, -m, qm)
        return jnp.concatenate([qm, jnp.zeros((104, QB), f32)], axis=0).astype(bf16)

    def finish_b(g, j, acc):
        on = _norm(acc, j)
        keep = (row24q >= OFF[j]) & (row24q < OFF[j] + DH)
        pltpu.store(otb.at[pl.ds(pl.multiple_of(72 * g + R0[j], 8), 24), :], on, mask=keep)
        return _lmin(acc, j), _absbits_max(on)

    def flag(pairs):
        l, fin = pairs[0]
        for a, b in pairs[1:]:
            l, fin = jnp.minimum(l, a), jnp.maximum(fin, b)
        lmin[...] = jnp.minimum(lmin[...], l)
        bad[...] = jnp.maximum(bad[...], fin)

    def group(qb, g, u):
        q0 = pl.multiple_of(qb * QB, QB)
        rows = pl.ds(pl.multiple_of(72 * g, 8), 72)
        flags = []
        if u == 0:
            l, fin = finish_b((g + G - 1) % G, 3, accc[...])
            flags.append((jnp.where(g > 0, l, BIG), jnp.where(g > 0, fin, 0)))
        st = {}
        bsteps, asteps = [], []
        for j in range(4):
            for cc in range(NC):
                def qk(j=j, cc=cc):
                    if cc == 0:
                        st['wb', j] = build_wb(qb, g, j)
                    return _dot(kb[cc * KC:(cc + 1) * KC, :], st['wb', j])

                def post(s):
                    return jnp.exp2(s).astype(bf16)

                def pv(p, j=j, cc=cc):
                    o = _dot(vb[j, :, cc * KC:(cc + 1) * KC], p)
                    st['acc', j] = o if cc == 0 else st['acc', j] + o
                    if cc == NC - 1:
                        if j == 3 and u == GU - 1:
                            accc[...] = st['acc', j]
                        else:
                            flags.append(finish_b(g, j, st['acc', j]))
                bsteps.append((qk, post, pv))
        for t in range(NT):
            def qk(t=t):
                ws = build_wa(qb, g, t)
                k0 = q0 + 128 * t
                return [_dot(kpa[g, pl.ds(pl.multiple_of(k0 + 64 * (r & 1), 64), 320), :], ws[r])
                        for r in range(4)]

            def post(ss):
                es = []
                for r in range(4):
                    e = jnp.exp2(ss[r])
                    es.append([jnp.where(m_lo, e[0:64], 0.0), e[64:128], e[128:192], e[192:256],
                               jnp.where(m_hi, e[256:320], 0.0)])
                ps = []
                for h in range(4):
                    e0, e1 = es[2 * (h >> 1)], es[2 * (h >> 1) + 1]
                    m0 = lblk64 == (h & 1)
                    pieces = [jnp.where(m0, e0[0], 0.0)]
                    for a in range(1, 5):
                        pieces.append(jnp.where(m0, e0[a], e1[a - 1]))
                    pieces.append(jnp.where(m0, 0.0, e1[4]))
                    ps.append(jnp.concatenate(pieces, axis=0).astype(bf16))
                return ps

            def pv(p, t=t):
                k0 = pl.multiple_of(q0 + 128 * t, 128)
                o, lm = [], None
                for j in range(4):
                    acc = _dot(va[g, j, :, pl.ds(k0, 384)], p[j])
                    on = _norm(acc, j)
                    o.append(on if j % 2 == 0 else pltpu.roll(on, 64, 1))
                    lm = _lmin(acc, j) if lm is None else jnp.minimum(lm, _lmin(acc, j))
                blk = _merge(o)
                ota[rows, 128 * t:128 * t + 128] = blk
                flags.append((lm, _absbits_max(blk)))
            asteps.append((qk, post, pv))
        steps = []
        for i, b in enumerate(bsteps):
            steps += [a for a, pos in zip(asteps, APOS) if pos == i]
            steps.append(b)
        n = len(steps)
        ps, pend = {}, []
        for i in range(n):
            ps[i] = steps[i][1](steps[i][0]())
            pend.append(i)
            lag = 2 if i >= n - 2 else 1
            while pend and pend[0] <= i - lag:
                k = pend.pop(0)
                steps[k][2](ps[k])
        for k in pend:
            steps[k][2](ps[k])
        flag(flags)

    def slow_head(qb, h):
        g, j = h // 4, h % 4
        q0 = qb * QB
        off = 2 * j
        win = pl.ds(pl.multiple_of(72 * g + 16 * j, 8), 24)
        keep = (row24q >= off) & (row24q < off + DH)
        isl = row24q == (off + DH) % 24

        def attend(scores, values, dst):
            m = lax.fori_loop(0, NC, lambda cc, m: jnp.maximum(m, jnp.max(scores(cc), axis=0, keepdims=True)),
                              jnp.full((1, QB), -jnp.inf, f32))
            acc = lax.fori_loop(0, NC, lambda cc, a: a + _dot(values(cc), jnp.exp2(scores(cc) - m).astype(bf16)),
                                jnp.zeros((24, QB), f32))
            l = jnp.sum(jnp.where(isl, acc, 0.0), axis=0, keepdims=True)
            pltpu.store(dst.at[win, :], acc * (1.0 / l), mask=keep)

        qw = pltpu.roll(qtb[win, qcols(qb)], (24 - off) % 24, 0)
        wb = jnp.concatenate([jnp.where(row24q < DH, qw, 0.0), jnp.zeros((104, QB), f32)], axis=0).astype(bf16)
        attend(lambda cc: _dot(kb[pl.ds(pl.multiple_of(cc * KC, KC), KC), :], wb),
               lambda cc: vb[j, :, pl.ds(pl.multiple_of(cc * KC, KC), KC)], otb)

        r128 = _rows(128, QB)
        qg = jnp.concatenate([qta[pl.ds(pl.multiple_of(72 * g, 8), 72), qcols(qb)], jnp.zeros((56, QB), f32)], axis=0)
        wa = jnp.where((r128 >= DH * j) & (r128 < DH * j + DH), qg, 0.0).astype(bf16)

        def scores_a(cc):
            s = _dot(kpa[g, pl.ds(pl.multiple_of(cc * KC + WIN, KC), KC), :], wa)
            dist = (q0 - cc * KC) + _lanes(KC, QB) - _rows(KC, QB)
            return jnp.where((dist >= 0) & (dist < WIN), s, -1e9 * LOG2E)

        attend(scores_a, lambda cc: va[g, j, :, pl.ds(pl.multiple_of(cc * KC + WIN, KC), KC)], ota)

    def slow_out_proj(qb, slot):
        def chunk(i, carry):
            w = woT[pl.ds(pl.multiple_of(128 * i, 128), 128), :]
            o = jnp.where(_rows(128, QB) + 128 * i < D, _dot(w, ota[...].astype(bf16)), _dot(w, otb[...].astype(bf16)))
            obuf[slot, :, pl.ds(pl.multiple_of(128 * i, 128), 128)] = o.astype(bf16).T
            return carry

        lax.fori_loop(0, 2 * D // 128, chunk, 0)
        cp_out(qb, slot).start()

    def cp_out(qb, slot):
        return pltpu.make_async_copy(obuf.at[slot], out_hbm.at[pl.ds(pl.multiple_of(qb * QB, QB), QB), :],
                                     out_sem.at[slot])

    def out_proj(qb, slot):
        oa = ota[...].astype(bf16)
        ob = otb[...].astype(bf16)
        for r in range(0, 2 * D, 128):
            if r + 128 <= D:
                o = _dot(woT[r:r + 128, :], oa)
            elif r >= D:
                o = _dot(woT[r:r + 128, :], ob)
            else:
                o = jnp.concatenate([_dot(woT[r:D, :], oa), _dot(woT[D:r + 128, :], ob)], axis=0)
            obuf[slot, :, r:r + 128] = o.astype(bf16).T
        cp_out(qb, slot).start()

    def qblock(qb, carry):
        slot = qb % 2

        @pl.when(qb >= 2)
        def _():
            cp_out(qb - 2, slot).wait()

        def gl(i, carry2):
            for u in range(GU):
                group(qb, i * GU + u, u)
            return carry2

        lax.fori_loop(0, G // GU, gl, 0)
        flag([finish_b(G - 1, 3, accc[...])])
        out_proj(qb, slot)

        unsafe = jnp.logical_or(jnp.max(bad[...]) >= 0x7F800000,
                                jnp.logical_not(jnp.min(lmin[...]) >= LMIN))

        @pl.when(unsafe)
        def _():
            cp_out(qb, slot).wait()

            def sl(h, carry2):
                slow_head(qb, h)
                return carry2

            lax.fori_loop(0, 4 * G, sl, 0)
            bad[...] = jnp.zeros(bad.shape, jnp.int32)
            lmin[...] = jnp.full(lmin.shape, BIG, f32)
            slow_out_proj(qb, slot)

        return carry

    lax.fori_loop(0, NQB, qblock, 0)
    cp_out(NQB - 2, 0).wait()
    cp_out(NQB - 1, 1).wait()


@jax.jit
def pallas_concat_heads__sliding_block__grouped_kv_mqa__prompt_kernel(
    A_x: jax.Array,
    A_wqkv: jax.Array,
    A_wo: jax.Array,
    B_x: jax.Array,
    B_wq: jax.Array,
    B_wk: jax.Array,
    B_wv: jax.Array,
    B_wo: jax.Array,
):
    scale = float(np.asarray(DH ** -0.5, dtype=A_x.dtype))
    scratch = [
        pltpu.VMEM((D, S), bf16),
        pltpu.VMEM((D, S), bf16),
        pltpu.VMEM((D, 3 * D), bf16),
        pltpu.VMEM((D, D), bf16),
        pltpu.VMEM((D, D), bf16),
        pltpu.VMEM((D, D), bf16),
        pltpu.VMEM((DH, D), bf16),
        pltpu.VMEM((DH, D), bf16),
        pltpu.VMEM((3 * D, D), bf16),
        pltpu.VMEM((D, D), bf16),
        pltpu.VMEM((2 * D, D), bf16),
        pltpu.VMEM((D, S), f32),
        pltpu.VMEM((D, S), f32),
        pltpu.VMEM((G, WIN + S, 128), bf16),
        pltpu.VMEM((G, 4, 24, WIN + S), f32),
        pltpu.VMEM((S, 128), bf16),
        pltpu.VMEM((4, 24, S), f32),
        pltpu.VMEM((G + 1, 8, 128), f32),
        pltpu.VMEM((G, 8, S), f32),
        pltpu.VMEM((G, 8, S), f32),
        pltpu.VMEM((2, 24, PB), f32),
        pltpu.VMEM((D, QB), f32),
        pltpu.VMEM((D, QB), f32),
        pltpu.VMEM((8, 128), jnp.int32),
        pltpu.VMEM((1, 128), f32),
        pltpu.VMEM((24, QB), f32),
        pltpu.VMEM((2, QB, 2 * D), bf16),
        pltpu.SemaphoreType.DMA((2 * NPB + 6,)),
        pltpu.SemaphoreType.DMA((2,)),
    ]
    anyspec = pl.BlockSpec(memory_space=pl.ANY)
    out = pl.pallas_call(
        functools.partial(_kernel, scale),
        out_shape=jax.ShapeDtypeStruct((S, 2 * D), A_x.dtype),
        in_specs=[anyspec] * 8,
        out_specs=anyspec,
        scratch_shapes=scratch,
        compiler_params=pltpu.CompilerParams(vmem_limit_bytes=100 * 1024 * 1024),
    )(A_x[0].T, A_wqkv, A_wo, B_x[0].T, B_wq, B_wk.T, B_wv.T, B_wo)
    return out[None]
```
